```python
import jax
import jax.numpy as jnp

def _softmax(x, axis=-1):
    return jax.nn.softmax(x, axis=axis)
def _gelu(x):
    return jax.nn.gelu(x, approximate=True)
def _silu(x):
    return jax.nn.silu(x)
def _sigmoid(x):
    return jax.nn.sigmoid(x)
def _layernorm(x, axis=-1, eps=1e-5):
    m = jnp.mean(x, axis=axis, keepdims=True)
    v = jnp.var(x, axis=axis, keepdims=True)
    return (x - m) / jnp.sqrt(v + eps)
def _scatter_add(tgt, idx, src, axis=0):
    return tgt.at[idx].add(src)
def _segment_sum(src, seg, n):
    return jax.ops.segment_sum(src, seg, n)
class _Rng:
    def __init__(self, key):
        self._k = key
    def _next(self):
        self._k, sub = jax.random.split(self._k)
        return sub
    def normal(self, shape):
        return jax.random.normal(self._next(), shape, dtype=jnp.bfloat16)
    def randint(self, lo, hi, shape):
        return jax.random.randint(self._next(), shape, lo, hi, dtype=jnp.int32)
    def uniform(self, shape, lo=0.0, hi=1.0):
        return jax.random.uniform(self._next(), shape, jnp.bfloat16, lo, hi)
    def permutation(self, n):
        return jax.random.permutation(self._next(), n)


kernel_name = 'gated_mix__sliding_local_dilated__glu_gated_reglu__prompt'

def setup_inputs():
    _rng = _Rng(jax.random.key(int.from_bytes(__import__("os").urandom(4), "little")))
    _w = (lambda a: (lambda t: t.astype(jnp.bfloat16) if jnp.issubdtype(t.dtype, jnp.floating) else t)(jnp.asarray(a)))
    def _A_setup():
        B, S, D = 1, 2048, 1024
        return {
            "x": _w((lambda *s: _rng.normal(s) * 0.05)(B, S, D)),
            "wqkv": _w((lambda *s: _rng.normal(s) * 0.05)(D, 3 * D)),
            "wo": _w((lambda *s: _rng.normal(s) * 0.05)(D, D)),
        }
    _A_in = _A_setup()

    def _B_setup():
        B, S, D, F = 1, 2048, 1024, 3584
        return {
            "x": _w((lambda *s: _rng.normal(s) * 0.05)(B, S, D)),
            "W_gate": _w((lambda *s: _rng.normal(s) * 0.05)(D, F) * (2.0 / D) ** 0.5),
            "W_up": _w((lambda *s: _rng.normal(s) * 0.05)(D, F) * (2.0 / D) ** 0.5),
            "W_down": _w((lambda *s: _rng.normal(s) * 0.05)(F, D) * (1.0 / F) ** 0.5),
        }
    _B_in = _B_setup()

    return {
        "A_x": _A_in["x"],
        "A_wqkv": _A_in["wqkv"],
        "A_wo": _A_in["wo"],
        "B_x": _B_in["x"],
        "B_W_gate": _B_in["W_gate"],
        "B_W_up": _B_in["W_up"],
        "B_W_down": _B_in["W_down"],
        "gate_w": _w((lambda *s: _rng.normal(s) * 0.05)(1024)),
    }

def reference(A_x, A_wqkv, A_wo, B_x, B_W_gate, B_W_up, B_W_down, gate_w):
    def _A_ref(x, wqkv, wo):
        B, S, D = x.shape
        H = 32; Dh = D // H
        W, dil = 8, 2
        qkv = (lambda x, *d: x.transpose(*d))((x @ wqkv).reshape(B, S, 3, H, Dh), 2, 0, 3, 1, 4)
        q, k, v = qkv[0], qkv[1], qkv[2]
        scale = Dh ** -0.5
        pos = jnp.arange(S)
        off = jnp.arange(W) * dil
        idx = pos[:, None] - off[None, :]
        mask = idx >= 0
        idx_c = jnp.where(mask, idx, 0).reshape(-1)
        kg = k[:, :, idx_c, :].reshape(B, H, S, W, Dh)
        vg = v[:, :, idx_c, :].reshape(B, H, S, W, Dh)
        logits = jnp.einsum("bhsd,bhswd->bhsw", q, kg) * scale
        logits = jnp.where(mask[None, None, :, :], logits, -1e9)
        attn = _softmax(logits, axis=-1)
        o = jnp.einsum("bhsw,bhswd->bhsd", attn, vg)
        return (lambda x, *d: x.transpose(*d))(o, 0, 2, 1, 3).reshape(B, S, D) @ wo

    def _B_ref(x, W_gate, W_up, W_down):
        gate = jnp.einsum("bsd,df->bsf", x, W_gate)
        up = jnp.einsum("bsd,df->bsf", x, W_up)
        gate = gate * (lambda x, dt: x.astype(dt))(gate > 0, gate.dtype)
        h = gate * up
        return jnp.einsum("bsf,fd->bsd", h, W_down)

    x = A_x
    g = _sigmoid((x * gate_w).sum(-1, keepdims=True))
    a = _A_ref(x, A_wqkv, A_wo)
    b = _B_ref(x, B_W_gate, B_W_up, B_W_down)
    return g * a + (1 - g) * b
```

```python
import functools
import numpy as np
import jax
import jax.numpy as jnp
from jax.experimental import pallas as pl
from jax.experimental.pallas import tpu as pltpu

S, D, F = 2048, 1024, 3584
H, DH, W, DIL = 32, 32, 8, 2
HALO = 16
f32, bf16, u32 = jnp.float32, jnp.bfloat16, jnp.uint32


def _perm_cols(w):
    x = pltpu.bitcast(w, u32)
    R = x.shape[0]
    lane = jax.lax.broadcasted_iota(jnp.int32, (R, 128), 1)
    G = lane >> 4
    hh, c = lane & 3, (lane >> 2) & 3
    a = []
    for g in range(8):
        j = (G - g) & 7
        idx = hh * 32 + 4 * j + c
        a.append(jnp.take_along_axis(x[:, 128 * g:128 * (g + 1)], idx, axis=1))
    a = [a[(-i) % 8] for i in range(8)]
    for b in (1, 2, 4):
        m = (G & b) != 0
        a = [jnp.where(m, a[(i - b) % 8], a[i]) for i in range(8)]
    out = []
    h = lane & 31
    c2 = lane >> 5
    for j in range(8):
        idx = 16 * ((j + (h >> 2)) & 7) + 4 * c2 + (h & 3)
        out.append(jnp.take_along_axis(a[j], idx, axis=1))
    return pltpu.bitcast(jnp.concatenate(out, axis=1), bf16)


def make(tm=128, f0=768, fc=512, rb=32, tp=128):
    nst = S // tm
    npro = S // tp
    FM = F - f0

    def kern(gw_ref, x_h, wqkv_h, wo_h, wg_h, wu_h, wd_h, o_ref,
             x_v, wqkv, wo, wg, wu, wd, wraw, woraw, tf, q_ref, k_ref, v_ref, o_scr, h_ref, b0_ref, xsem, sems):
        i = pl.program_id(0)

        def cp_x(r): return pltpu.make_async_copy(x_h.at[pl.ds(r*tp, tp), :], x_v.at[pl.ds(r*tp, tp), :], xsem.at[r])
        c_g0 = pltpu.make_async_copy(wg_h.at[:, :f0], wg.at[:, :f0], sems.at[0])
        c_u0 = pltpu.make_async_copy(wu_h.at[:, :f0], wu.at[:, :f0], sems.at[1])
        c_d0 = pltpu.make_async_copy(wd_h.at[:f0, :], wd.at[:f0, :], sems.at[2])
        c_qkv = pltpu.make_async_copy(wqkv_h, wraw, sems.at[3])
        c_os = [pltpu.make_async_copy(wo_h.at[:, n*128:(n+1)*128], woraw.at[n], sems.at[8+n]) for n in range(8)]
        c_g1 = pltpu.make_async_copy(wg_h.at[:, f0:], wg.at[:, f0:], sems.at[5])
        c_u1 = pltpu.make_async_copy(wu_h.at[:, f0:], wu.at[:, f0:], sems.at[6])
        c_d1 = pltpu.make_async_copy(wd_h.at[f0:, :], wd.at[f0:, :], sems.at[7])

        def pro_ffn(r, first=False):
            r0 = r * tp if first else pl.multiple_of(r * tp, tp)
            cp_x(r).wait()
            x = x_v[pl.ds(r0, tp), :]
            if first: c_g0.wait()
            g = jnp.dot(x, wg[:, :f0], preferred_element_type=f32)
            if first: c_u0.wait()
            u = jnp.dot(x, wu[:, :f0], preferred_element_type=f32)
            h = (jnp.maximum(g, 0.0) * u).astype(bf16)
            if first: c_d0.wait()
            b0_ref[pl.ds(r0, tp), :] = jnp.dot(h, wd[:f0, :], preferred_element_type=f32)

        def prep(n):
            r0 = pl.multiple_of(n * 128, 128)
            for t in range(3):
                wqkv[pl.ds(r0, 128), t*D:(t+1)*D] = _perm_cols(wraw[pl.ds(r0, 128), t*D:(t+1)*D])
            tf[...] = woraw[n].astype(f32)
            for d in range(0, DH, 4):
                blk = jnp.concatenate([tf[pl.ds(d + e, H, stride=DH), :] for e in range(4)], axis=0)
                wo[n, d*H:(d+4)*H, :] = blk.astype(bf16)

        @pl.when(i == 0)
        def _():
            cp_x(0).start(); c_g0.start(); c_u0.start(); c_d0.start()
            cp_x(1).start(); cp_x(2).start()
            c_qkv.start()
            for c in c_os: c.start()
            for r in range(3, npro): cp_x(r).start()
            c_g1.start(); c_u1.start(); c_d1.start()
            k_ref[0:HALO, :] = jnp.zeros((HALO, D), f32)
            v_ref[0:HALO, :] = jnp.zeros((HALO, D), f32)
            pro_ffn(0, True)
            na = npro - 8
            def la(r, c):
                pro_ffn(r); return c
            jax.lax.fori_loop(1, na, la, 0)
            c_qkv.wait()
            for c in c_os: c.wait()
            def lb(r, c):
                pro_ffn(r); prep(r - na); return c
            jax.lax.fori_loop(na, npro, lb, 0)
            c_g1.wait(); c_u1.wait(); c_d1.wait()

        row0 = pl.multiple_of(i * tm, tm)
        x = x_v[pl.ds(row0, tm), :]
        q_ref[...] = jnp.dot(x, wqkv[:, 0:D], preferred_element_type=f32)
        k_ref[HALO:, :] = jnp.dot(x, wqkv[:, D:2*D], preferred_element_type=f32)
        v_ref[HALO:, :] = jnp.dot(x, wqkv[:, 2*D:], preferred_element_type=f32)

        def attn(r0):
            scale = DH ** -0.5
            q = q_ref[r0:r0+rb, :]
            ls = []
            for w in range(W):
                p = q * k_ref[HALO + r0 - DIL*w:HALO + r0 + rb - DIL*w, :]
                s = p[:, 0:128]
                for j in range(1, 8):
                    s = s + p[:, j*128:(j+1)*128]
                s = s + pltpu.roll(s, 64, 1)
                s = s + pltpu.roll(s, 32, 1)
                s = s * scale
                if r0 < DIL*w:
                    row = jax.lax.broadcasted_iota(jnp.int32, (rb, 128), 0) + (r0 + i * tm)
                    s = jnp.where(row >= DIL*w, s, -1e9)
                ls.append(s)
            m = ls[0]
            for w in range(1, W): m = jnp.maximum(m, ls[w])
            es = [jnp.exp(l - m) for l in ls]
            den = es[0]
            for w in range(1, W): den = den + es[w]
            inv = 1.0 / den
            ps = [e * inv for e in es]
            for j in range(8):
                acc = ps[0] * v_ref[HALO + r0:HALO + r0 + rb, j*128:(j+1)*128]
                for w in range(1, W):
                    acc = acc + ps[w] * v_ref[HALO + r0 - DIL*w:HALO + r0 + rb - DIL*w, j*128:(j+1)*128]
                o_scr[r0:r0+rb, j*128:(j+1)*128] = acc.astype(bf16)

        chunks = [(c0, min(c0 + fc, F)) for c0 in range(f0, F, fc)]
        rbs = list(range(0, tm, rb))
        for ci, (c0, c1) in enumerate(chunks):
            g = jnp.dot(x, wg[:, c0:c1], preferred_element_type=f32)
            u = jnp.dot(x, wu[:, c0:c1], preferred_element_type=f32)
            h_ref[:, c0-f0:c1-f0] = (jnp.maximum(g, 0.0) * u).astype(bf16)
            lo = ci * len(rbs) // len(chunks); hi = (ci + 1) * len(rbs) // len(chunks)
            for r0 in rbs[lo:hi]: attn(r0)
        k_ref[0:HALO, :] = k_ref[tm:tm+HALO, :]
        v_ref[0:HALO, :] = v_ref[tm:tm+HALO, :]
        b = b0_ref[pl.ds(row0, tm), :] + jnp.dot(h_ref[...], wd[f0:, :], preferred_element_type=f32)
        o = o_scr[...]
        a = jnp.concatenate([jnp.dot(o, wo[n], preferred_element_type=f32) for n in range(8)], axis=1)
        xg = x.astype(f32) * gw_ref[...].astype(f32)
        g = jax.nn.sigmoid(jnp.sum(xg, axis=-1, keepdims=True))
        o_ref[...] = (g * a + (1.0 - g) * b).astype(o_ref.dtype)

    @jax.jit
    def fn(A_x, A_wqkv, A_wo, B_x, B_W_gate, B_W_up, B_W_down, gate_w):
        anyspec = pl.BlockSpec(memory_space=pl.ANY)
        out = pl.pallas_call(
            kern, grid=(nst,),
            in_specs=[pl.BlockSpec((1, D), lambda i: (0, 0))] + [anyspec] * 6,
            out_specs=pl.BlockSpec((tm, D), lambda i: (i, 0)),
            out_shape=jax.ShapeDtypeStruct((S, D), A_x.dtype),
            scratch_shapes=[
                pltpu.VMEM((S, D), bf16),
                pltpu.VMEM((D, 3*D), bf16), pltpu.VMEM((8, D, 128), bf16),
                pltpu.VMEM((D, F), bf16), pltpu.VMEM((D, F), bf16), pltpu.VMEM((F, D), bf16),
                pltpu.VMEM((D, 3*D), bf16), pltpu.VMEM((8, D, 128), bf16), pltpu.VMEM((D, 128), f32),
                pltpu.VMEM((tm, D), f32), pltpu.VMEM((HALO + tm, D), f32), pltpu.VMEM((HALO + tm, D), f32),
                pltpu.VMEM((tm, D), bf16), pltpu.VMEM((tm, FM), bf16), pltpu.VMEM((S, D), f32),
                pltpu.SemaphoreType.DMA((npro,)), pltpu.SemaphoreType.DMA((16,)),
            ],
            compiler_params=pltpu.CompilerParams(dimension_semantics=("arbitrary",), vmem_limit_bytes=100 * 2**20),
        )(gate_w.reshape(1, D), A_x.reshape(S, D), A_wqkv, A_wo, B_W_gate, B_W_up, B_W_down)
        return out.reshape(1, S, D)
    return fn


pallas_gated_mix__sliding_local_dilated__glu_gated_reglu__prompt_kernel = make()
```
